```python
import jax
import jax.numpy as jnp

def _softmax(x, axis=-1):
    return jax.nn.softmax(x, axis=axis)

def _gelu(x):
    return jax.nn.gelu(x, approximate=True)

def _silu(x):
    return jax.nn.silu(x)

def _sigmoid(x):
    return jax.nn.sigmoid(x)

def _layernorm(x, axis=-1, eps=1e-05):
    m = jnp.mean(x, axis=axis, keepdims=True)
    v = jnp.var(x, axis=axis, keepdims=True)
    return (x - m) / jnp.sqrt(v + eps)

def _scatter_add(tgt, idx, src, axis=0):
    return tgt.at[idx].add(src)

def _segment_sum(src, seg, n):
    return jax.ops.segment_sum(src, seg, n)

class _Rng:

    def __init__(self, key):
        self._k = key

    def _next(self):
        self._k, sub = jax.random.split(self._k)
        return sub

    def normal(self, shape):
        return jax.random.normal(self._next(), shape, dtype=jnp.bfloat16)

    def randint(self, lo, hi, shape):
        return jax.random.randint(self._next(), shape, lo, hi, dtype=jnp.int32)

    def uniform(self, shape, lo=0.0, hi=1.0):
        return jax.random.uniform(self._next(), shape, jnp.bfloat16, lo, hi)

    def permutation(self, n):
        return jax.random.permutation(self._next(), n)
kernel_name = 'adaLN_cond__compressed_kv_cla__dense_activation_relu__decode'

def setup_inputs():
    _rng = _Rng(jax.random.key(int.from_bytes(__import__("os").urandom(4), "little")))
    _w = lambda a: (lambda t: t.astype(jnp.bfloat16) if jnp.issubdtype(t.dtype, jnp.floating) else t)(jnp.asarray(a))

    def _A_setup():
        B, H, Sq, Sk, D, M = (8, 32, 1, 4096, 128, 512)
        Dc = 4 * D
        return {'x': _w((lambda *s: _rng.normal(s) * 0.05)(B, Sq, M)), 'c_kv': _w((lambda *s: _rng.normal(s) * 0.05)(B, Sk, Dc)), 'w_q': _w((lambda *s: _rng.normal(s) * 0.05)(M, H, D) * M ** (-0.5)), 'w_uk': _w((lambda *s: _rng.normal(s) * 0.05)(Dc, H, D) * Dc ** (-0.5)), 'w_uv': _w((lambda *s: _rng.normal(s) * 0.05)(Dc, H, D) * Dc ** (-0.5)), 'w_o': _w((lambda *s: _rng.normal(s) * 0.05)(H, D, M) * (H * D) ** (-0.5))}
    _A_in = _A_setup()

    def _B_setup():
        B, S, D, Dff = (8, 1, 512, 1792)
        return {'x': _w((lambda *s: _rng.normal(s) * 0.05)(B, S, D)), 'w1': _w((lambda *s: _rng.normal(s) * 0.05)(D, Dff)), 'w2': _w((lambda *s: _rng.normal(s) * 0.05)(Dff, D))}
    _B_in = _B_setup()
    return {'A_x': _A_in['x'], 'A_c_kv': _A_in['c_kv'], 'A_w_q': _A_in['w_q'], 'A_w_uk': _A_in['w_uk'], 'A_w_uv': _A_in['w_uv'], 'A_w_o': _A_in['w_o'], 'B_x': _B_in['x'], 'B_w1': _B_in['w1'], 'B_w2': _B_in['w2'], 'c': _w((lambda *s: _rng.normal(s) * 0.05)(8, 512)), 'w_mod': _w((lambda *s: _rng.normal(s) * 0.05)(512, 6 * 512) * 512 ** (-0.5))}

def reference(A_x, A_c_kv, A_w_q, A_w_uk, A_w_uv, A_w_o, B_x, B_w1, B_w2, c, w_mod):

    def _A_ref(x, c_kv, w_q, w_uk, w_uv, w_o):
        B, Sq, M = (x.shape[0], x.shape[1], x.shape[2])
        Sk = c_kv.shape[1]
        H, D = (w_q.shape[1], w_q.shape[2])
        q = jnp.einsum('bqm,mhd->bhqd', x, w_q)
        k = jnp.einsum('bkc,chd->bhkd', c_kv, w_uk)
        v = jnp.einsum('bkc,chd->bhkd', c_kv, w_uv)
        scores = jnp.einsum('bhqd,bhkd->bhqk', q, k) * D ** (-0.5)
        off = Sk - Sq
        qi = jnp.arange(Sq)[:, None]
        kj = jnp.arange(Sk)[None, :]
        cmask = kj <= qi + off
        scores = jnp.where(cmask[None, None], scores, -1000000000.0)
        p = _softmax(scores, axis=-1)
        ctx = jnp.einsum('bhqk,bhkd->bhqd', p, v)
        return jnp.einsum('bhqd,hdm->bqm', ctx, w_o)

    def _B_ref(x, w1, w2):
        h = jnp.einsum('bsd,df->bsf', x, w1)
        zero = jnp.zeros_like(h)
        h = jnp.maximum(h, zero)
        return jnp.einsum('bsf,fd->bsd', h, w2)
    x = A_x
    mod = (_silu(c) @ w_mod).reshape(c.shape[0], 6, 1, -1)
    sa, ca, ga, sb, cb, gb = (mod[:, 0].copy(), mod[:, 1].copy(), mod[:, 2].copy(), mod[:, 3].copy(), mod[:, 4].copy(), mod[:, 5].copy())
    h = _layernorm(x, axis=-1) * (1 + ca) + sa
    x = x + ga * _A_ref(h, A_c_kv, A_w_q, A_w_uk, A_w_uv, A_w_o)
    h = _layernorm(x, axis=-1) * (1 + cb) + sb
    x = x + gb * _B_ref(h, B_w1, B_w2)
    return x
```

```python
import jax
import jax.numpy as jnp
from jax import lax
import jax.experimental.pallas as pl
import jax.experimental.pallas.tpu as pltpu

B = 8
SK = 4096
M = 512
DC = 512
H = 32
D = 128
DFF = 1792
NCT = DC // 128
EPS = 1e-05
SCALE = float(D) ** -0.5

F32 = jnp.float32
BF16 = jnp.bfloat16
U32 = jnp.uint32


def _dot(a, b):
    return jnp.dot(a, b, preferred_element_type=F32)


def _dot_nt(a, b):
    return lax.dot_general(a, b, (((1,), (1,)), ((), ())),
                           preferred_element_type=F32)


def _layernorm(x):
    m = jnp.mean(x, axis=-1, keepdims=True)
    xc = x - m
    v = jnp.mean(xc * xc, axis=-1, keepdims=True)
    return xc / jnp.sqrt(v + EPS)


def _head_pair(w32_ref, j):
    rows = w32_ref.shape[0] // (H // 2)
    words = w32_ref[pl.ds(j, rows, stride=H // 2), :]
    lo = lax.bitcast_convert_type(words << 16, F32).astype(BF16)
    hi = lax.bitcast_convert_type(words & jnp.uint32(0xFFFF0000), F32).astype(BF16)
    return lo, hi


def _kernel(x_hbm, ckv_hbm, wq_hbm, wuk_hbm, wuv_hbm, wo_hbm, w1_hbm, w2_hbm,
            c_hbm, wmod_hbm,
            o_ref,
            x_v, c_v, wmod_v, wq_v, wuk_v, ckv_v, wuv_v, wo_v, w1_v, w2_v,
            q_s, qa_s, cc_s, ctx_s, sems):
    copies = {}
    order = []

    def add(name, src, dst):
        copies[name] = pltpu.make_async_copy(src, dst, sems.at[len(order)])
        order.append(name)

    add("c", c_hbm, c_v)
    add("x", x_hbm, x_v)
    add("wmod", wmod_hbm, wmod_v)
    add("wq", wq_hbm.bitcast(U32), wq_v)
    add("wuk", wuk_hbm.bitcast(U32), wuk_v)
    kv_sem0 = len(order)
    for b in range(B):
        add(("kv", b), ckv_hbm.at[b], ckv_v.at[b])
    add("wuv", wuv_hbm.bitcast(U32), wuv_v)
    add("wo", wo_hbm, wo_v)
    add("w1", w1_hbm, w1_v)
    add("w2", w2_hbm, w2_v)
    for name in order:
        copies[name].start()

    copies["c"].wait()
    copies["x"].wait()
    c = c_v[...].astype(F32)
    sc = (c * jax.nn.sigmoid(c)).astype(BF16)
    x0 = x_v[...].reshape(B, M).astype(F32)
    ln0 = _layernorm(x0)
    copies["wmod"].wait()
    mod = _dot(sc, wmod_v[...])
    sa, ca, ga, sb, cb, gb = [mod[:, i * M:(i + 1) * M] for i in range(6)]
    h1 = (ln0 * (1.0 + ca) + sa).astype(BF16)

    copies["wq"].wait()
    wq32 = wq_v

    def q_body(j, carry):
        lo, hi = _head_pair(wq32, j)
        q_s[2 * j] = _dot(h1, lo).astype(BF16)
        q_s[2 * j + 1] = _dot(h1, hi).astype(BF16)
        return carry

    lax.fori_loop(0, H // 2, q_body, 0)

    copies["wuk"].wait()
    wuk32 = wuk_v

    def qa_body(j, carry):
        lo, hi = _head_pair(wuk32, j)
        r0 = pl.multiple_of(2 * j * B, B)
        r1 = pl.multiple_of((2 * j + 1) * B, B)
        a0 = _dot_nt(q_s[2 * j], lo) * SCALE
        a1 = _dot_nt(q_s[2 * j + 1], hi) * SCALE
        for t in range(NCT):
            qa_s[t, pl.ds(r0, B), :] = a0[:, t * 128:(t + 1) * 128]
            qa_s[t, pl.ds(r1, B), :] = a1[:, t * 128:(t + 1) * 128]
        return carry

    lax.fori_loop(0, H // 2, qa_body, 0)

    def attn_body(b, carry):
        pltpu.make_async_copy(ckv_hbm.at[b], ckv_v.at[b], sems.at[kv_sem0 + b]).wait()
        qa = jnp.concatenate(
            [qa_s[t, pl.ds(b, H, stride=B), :] for t in range(NCT)],
            axis=-1).astype(BF16)
        kv = ckv_v[b]
        s = _dot_nt(qa, kv)
        m = jnp.max(s, axis=-1, keepdims=True)
        p = jnp.exp(s - m)
        l = jnp.sum(p, axis=-1, keepdims=True)
        cc = _dot(p.astype(BF16), kv) / l
        r0 = pl.multiple_of(b * H, H)
        for t in range(NCT):
            cc_s[t, pl.ds(r0, H), :] = cc[:, t * 128:(t + 1) * 128]
        return carry

    lax.fori_loop(0, B, attn_body, 0)

    copies["wuv"].wait()
    wuv32 = wuv_v

    def ctx_body(j, carry):
        lo, hi = _head_pair(wuv32, j)
        c0 = jnp.concatenate(
            [cc_s[t, pl.ds(2 * j, B, stride=H), :] for t in range(NCT)],
            axis=-1).astype(BF16)
        c1 = jnp.concatenate(
            [cc_s[t, pl.ds(2 * j + 1, B, stride=H), :] for t in range(NCT)],
            axis=-1).astype(BF16)
        ctx_s[2 * j] = _dot(c0, lo).astype(BF16)
        ctx_s[2 * j + 1] = _dot(c1, hi).astype(BF16)
        return carry

    lax.fori_loop(0, H // 2, ctx_body, 0)

    copies["wo"].wait()
    ctx = jnp.concatenate([ctx_s[h] for h in range(H)], axis=-1)
    attn = _dot(ctx, wo_v[...])
    x1 = x0 + ga * attn

    h2 = (_layernorm(x1) * (1.0 + cb) + sb).astype(BF16)
    copies["w1"].wait()
    f = jnp.maximum(_dot(h2, w1_v[...]), 0.0).astype(BF16)
    copies["w2"].wait()
    y = _dot(f, w2_v[...])
    x2 = x1 + gb * y
    o_ref[...] = x2.astype(o_ref.dtype).reshape(o_ref.shape)


@jax.jit
def pallas_adaLN_cond__compressed_kv_cla__dense_activation_relu__decode_kernel(
    A_x: jax.Array,
    A_c_kv: jax.Array,
    A_w_q: jax.Array,
    A_w_uk: jax.Array,
    A_w_uv: jax.Array,
    A_w_o: jax.Array,
    B_x: jax.Array,
    B_w1: jax.Array,
    B_w2: jax.Array,
    c: jax.Array,
    w_mod: jax.Array,
):
    del B_x
    wq2 = A_w_q.reshape(M * H, D)
    wuk2 = A_w_uk.reshape(DC * H, D)
    wuv2 = A_w_uv.reshape(DC * H, D)
    wo2 = A_w_o.reshape(H * D, M)

    any_spec = pl.BlockSpec(memory_space=pl.ANY)
    n_dma = 9 + B
    scratch = [
        pltpu.VMEM((B, 1, M), BF16),
        pltpu.VMEM((B, M), BF16),
        pltpu.VMEM((M, 6 * M), BF16),
        pltpu.VMEM((M * H // 2, D), U32),
        pltpu.VMEM((DC * H // 2, D), U32),
        pltpu.VMEM((B, SK, DC), BF16),
        pltpu.VMEM((DC * H // 2, D), U32),
        pltpu.VMEM((H * D, M), BF16),
        pltpu.VMEM((M, DFF), BF16),
        pltpu.VMEM((DFF, M), BF16),
        pltpu.VMEM((H, B, D), BF16),
        pltpu.VMEM((NCT, H * B, 128), F32),
        pltpu.VMEM((NCT, B * H, 128), F32),
        pltpu.VMEM((H, B, D), BF16),
        pltpu.SemaphoreType.DMA((n_dma,)),
    ]
    return pl.pallas_call(
        _kernel,
        out_shape=jax.ShapeDtypeStruct((B, 1, M), BF16),
        in_specs=[any_spec] * 10,
        out_specs=pl.BlockSpec(memory_space=pltpu.VMEM),
        scratch_shapes=scratch,
        compiler_params=pltpu.CompilerParams(vmem_limit_bytes=100 * 1024 * 1024),
    )(A_x, A_c_kv, wq2, wuk2, wuv2, wo2, B_w1, B_w2, c, w_mod)
```

```python
import jax
import jax.numpy as jnp
from jax import lax
import jax.experimental.pallas as pl
import jax.experimental.pallas.tpu as pltpu

B = 8
SK = 4096
M = 512
DC = 512
H = 32
D = 128
DFF = 1792
NCT = DC // 128
NSEM = 3
W2A = 1536
EPS = 1e-05
SCALE = float(D) ** -0.5

F32 = jnp.float32
BF16 = jnp.bfloat16
U32 = jnp.uint32


def _dot(a, b):
    return jnp.dot(a, b, preferred_element_type=F32)


def _dot_nt(a, b):
    return lax.dot_general(a, b, (((1,), (1,)), ((), ())),
                           preferred_element_type=F32)


def _layernorm(x):
    m = jnp.mean(x, axis=-1, keepdims=True)
    xc = x - m
    v = jnp.mean(xc * xc, axis=-1, keepdims=True)
    return xc / jnp.sqrt(v + EPS)


def _head_pair(w32_ref, j):
    rows = w32_ref.shape[0] // (H // 2)
    words = w32_ref[pl.ds(j, rows, stride=H // 2), :]
    lo = lax.bitcast_convert_type(words << 16, F32).astype(BF16)
    hi = lax.bitcast_convert_type(words & jnp.uint32(0xFFFF0000), F32).astype(BF16)
    return lo, hi


def _kernel(x_hbm, ckv_hbm, wq_hbm, wuk_hbm, wuv_hbm, wo_hbm, w1_hbm, w2_hbm,
            c_hbm, wmod_hbm,
            o_ref,
            x_v, c_v, wmod_v, wq_v, wuk_v, ckv_v, wuv_v, wo_v, w1_v, w2_v,
            q_s, qa_s, cc_s, ctx_s, acc_s, sems):
    groups = [
        [(c_hbm, c_v), (x_hbm, x_v), (wmod_hbm, wmod_v)],
        [(wq_hbm.bitcast(U32), wq_v)],
        [(wuk_hbm.bitcast(U32), wuk_v)],
    ]
    KV0 = len(groups)
    groups += [[(ckv_hbm.at[b], ckv_v.at[b])] for b in range(B)]
    WUV = len(groups)
    groups += [
        [(wuv_hbm.bitcast(U32), wuv_v)],
        [(wo_hbm, wo_v)],
        [(w1_hbm, w1_v)],
        [(w2_hbm.at[pl.ds(0, W2A)], w2_v.at[pl.ds(0, W2A)])],
        [(w2_hbm.at[pl.ds(W2A, DFF - W2A)], w2_v.at[pl.ds(W2A, DFF - W2A)])],
    ]

    def copies(g):
        return [pltpu.make_async_copy(src, dst, sems.at[g % NSEM])
                for src, dst in groups[g]]

    def start(g):
        if g < len(groups):
            for cp in copies(g):
                cp.start()

    def wait(g):
        for cp in copies(g):
            cp.wait()

    def wait_and_refill(g):
        wait(g)
        start(g + NSEM)

    for g in range(NSEM):
        start(g)

    wait_and_refill(0)
    c = c_v[...].astype(F32)
    sc = (c * jax.nn.sigmoid(c)).astype(BF16)
    x0 = x_v[...].astype(F32)
    ln0 = _layernorm(x0)
    mod = _dot(sc, wmod_v[...])
    sa, ca, ga, sb, cb, gb = [mod[:, i * M:(i + 1) * M] for i in range(6)]
    h1 = (ln0 * (1.0 + ca) + sa).astype(BF16)

    wait_and_refill(1)
    wq32 = wq_v

    def q_body(j, carry):
        lo, hi = _head_pair(wq32, j)
        q_s[2 * j] = _dot(h1, lo).astype(BF16)
        q_s[2 * j + 1] = _dot(h1, hi).astype(BF16)
        return carry

    lax.fori_loop(0, H // 2, q_body, 0)

    wait_and_refill(2)
    wuk32 = wuk_v

    def qa_body(j, carry):
        lo, hi = _head_pair(wuk32, j)
        r0 = pl.multiple_of(2 * j * B, B)
        r1 = pl.multiple_of((2 * j + 1) * B, B)
        a0 = _dot_nt(q_s[2 * j], lo) * SCALE
        a1 = _dot_nt(q_s[2 * j + 1], hi) * SCALE
        for t in range(NCT):
            qa_s[t, pl.ds(r0, B), :] = a0[:, t * 128:(t + 1) * 128]
            qa_s[t, pl.ds(r1, B), :] = a1[:, t * 128:(t + 1) * 128]
        return carry

    lax.fori_loop(0, H // 2, qa_body, 0)

    def attn_body(b, carry):
        sem = sems.at[(KV0 + b) % NSEM]
        pltpu.make_async_copy(ckv_hbm.at[b], ckv_v.at[b], sem).wait()

        @pl.when(b + NSEM < B)
        def _():
            nb = b + NSEM
            pltpu.make_async_copy(ckv_hbm.at[nb], ckv_v.at[nb], sem).start()

        for i in range(NSEM):
            @pl.when(b == B - NSEM + i)
            def _():
                start(WUV + i)

        qa = jnp.concatenate(
            [qa_s[t, pl.ds(b, H, stride=B), :] for t in range(NCT)],
            axis=-1).astype(BF16)
        kv = ckv_v[b]
        s = _dot_nt(qa, kv)
        m = jnp.max(s, axis=-1, keepdims=True)
        p = jnp.exp(s - m)
        l = jnp.sum(p, axis=-1, keepdims=True)
        cc = _dot(p.astype(BF16), kv) / l
        r0 = pl.multiple_of(b * H, H)
        for t in range(NCT):
            cc_s[t, pl.ds(r0, H), :] = cc[:, t * 128:(t + 1) * 128]
        return carry

    lax.fori_loop(0, B, attn_body, 0)

    wait_and_refill(WUV)
    wuv32 = wuv_v

    def ctx_body(j, carry):
        lo, hi = _head_pair(wuv32, j)
        c0 = jnp.concatenate(
            [cc_s[t, pl.ds(2 * j, B, stride=H), :] for t in range(NCT)],
            axis=-1).astype(BF16)
        c1 = jnp.concatenate(
            [cc_s[t, pl.ds(2 * j + 1, B, stride=H), :] for t in range(NCT)],
            axis=-1).astype(BF16)
        ctx_s[2 * j] = _dot(c0, lo).astype(BF16)
        ctx_s[2 * j + 1] = _dot(c1, hi).astype(BF16)
        return carry

    lax.fori_loop(0, H // 2, ctx_body, 0)

    wait_and_refill(WUV + 1)
    ctx = jnp.concatenate([ctx_s[h] for h in range(H)], axis=-1)
    attn = _dot(ctx, wo_v[...])
    x1 = x0 + ga * attn

    h2 = (_layernorm(x1) * (1.0 + cb) + sb).astype(BF16)
    wait_and_refill(WUV + 2)
    f = jnp.maximum(_dot(h2, w1_v[...]), 0.0).astype(BF16)
    wait_and_refill(WUV + 3)
    acc_s[...] = x1 + gb * _dot(f[:, :W2A], w2_v[pl.ds(0, W2A), :])
    wait_and_refill(WUV + 4)
    x2 = acc_s[...] + gb * _dot(f[:, W2A:], w2_v[pl.ds(W2A, DFF - W2A), :])
    o_ref[...] = x2.astype(o_ref.dtype)


@jax.jit
def pallas_adaLN_cond__compressed_kv_cla__dense_activation_relu__decode_kernel(
    A_x: jax.Array,
    A_c_kv: jax.Array,
    A_w_q: jax.Array,
    A_w_uk: jax.Array,
    A_w_uv: jax.Array,
    A_w_o: jax.Array,
    B_x: jax.Array,
    B_w1: jax.Array,
    B_w2: jax.Array,
    c: jax.Array,
    w_mod: jax.Array,
):
    del B_x
    wq2 = A_w_q.reshape(M * H, D)
    wuk2 = A_w_uk.reshape(DC * H, D)
    wuv2 = A_w_uv.reshape(DC * H, D)
    wo2 = A_w_o.reshape(H * D, M)

    any_spec = pl.BlockSpec(memory_space=pl.ANY)
    scratch = [
        pltpu.VMEM((B, M), BF16),
        pltpu.VMEM((B, M), BF16),
        pltpu.VMEM((M, 6 * M), BF16),
        pltpu.VMEM((M * H // 2, D), U32),
        pltpu.VMEM((DC * H // 2, D), U32),
        pltpu.VMEM((B, SK, DC), BF16),
        pltpu.VMEM((DC * H // 2, D), U32),
        pltpu.VMEM((H * D, M), BF16),
        pltpu.VMEM((M, DFF), BF16),
        pltpu.VMEM((DFF, M), BF16),
        pltpu.VMEM((H, B, D), BF16),
        pltpu.VMEM((NCT, H * B, 128), F32),
        pltpu.VMEM((NCT, B * H, 128), F32),
        pltpu.VMEM((H, B, D), BF16),
        pltpu.VMEM((B, M), F32),
        pltpu.SemaphoreType.DMA((NSEM,)),
    ]
    out = pl.pallas_call(
        _kernel,
        out_shape=jax.ShapeDtypeStruct((B, M), BF16),
        in_specs=[any_spec] * 10,
        out_specs=pl.BlockSpec(memory_space=pltpu.VMEM),
        scratch_shapes=scratch,
        compiler_params=pltpu.CompilerParams(vmem_limit_bytes=100 * 1024 * 1024),
    )(A_x.reshape(B, M), A_c_kv, wq2, wuk2, wuv2, wo2, B_w1, B_w2, c, w_mod)
    return out.reshape(B, 1, M)
```

```python
import jax
import jax.numpy as jnp
from jax import lax
import jax.experimental.pallas as pl
import jax.experimental.pallas.tpu as pltpu

B = 8
SK = 4096
M = 512
DC = 512
H = 32
D = 128
DFF = 1792
NCT = DC // 128
NP = H // 2
EPS = 1e-05
SCALE = float(D) ** -0.5

NSEM = 3
W2A = 1536
PITCH = 24
UNROLL = 4
SIDE = 6
SIDE_C = 30
C_MAIN = DC - SIDE * SIDE_C

F32 = jnp.float32
BF16 = jnp.bfloat16
U32 = jnp.uint32


def _dot(a, b):
    return jnp.dot(a, b, preferred_element_type=F32)


def _dot_nt(a, b):
    return lax.dot_general(a, b, (((1,), (1,)), ((), ())),
                           preferred_element_type=F32)


def _layernorm(x):
    m = jnp.mean(x, axis=-1, keepdims=True)
    xc = x - m
    v = jnp.mean(xc * xc, axis=-1, keepdims=True)
    return xc / jnp.sqrt(v + EPS)


def _head_pair(w_ref, j):
    rows = w_ref.shape[0]
    flat = w_ref.reshape(rows * PITCH, D)
    words = flat[pl.ds(j, rows, stride=PITCH), :]
    lo = lax.bitcast_convert_type(words << 16, F32).astype(BF16)
    hi = lax.bitcast_convert_type(words & jnp.uint32(0xFFFF0000), F32).astype(BF16)
    return lo, hi


def _kernel(x_hbm, ckv_hbm, wq_hbm, wuk_hbm, wuv_hbm, wo_hbm, w1_hbm, w2_hbm,
            c_hbm, wmod_hbm,
            o_ref,
            x_v, c_v, wmod_v, wq_v, wuk_v, ckv_v, wuv_v, wo_v, w1_v, w2_v,
            q_s, qa_s, cc_s, ctx_s, acc_s, sems, side_buf, side_sem):
    wuv32 = wuv_hbm.bitcast(U32)

    def slabs(v, r0, n):
        return v.at[pl.ds(r0, n), pl.ds(0, NP), :]

    groups = [
        [(c_hbm, c_v), (x_hbm, x_v), (wmod_hbm, wmod_v)],
        [(wq_hbm.bitcast(U32), slabs(wq_v, 0, M))],
        [(wuk_hbm.bitcast(U32), slabs(wuk_v, 0, DC))],
    ]
    KV0 = len(groups)
    groups += [[(ckv_hbm.at[b], ckv_v.at[b])] for b in range(B)]
    WUV = len(groups)
    groups += [
        [(wuv32.at[pl.ds(0, C_MAIN)], slabs(wuv_v, 0, C_MAIN))],
        [(wo_hbm, wo_v)],
        [(w1_hbm, w1_v)],
        [(w2_hbm.at[pl.ds(0, W2A)], w2_v.at[pl.ds(0, W2A)])],
        [(w2_hbm.at[pl.ds(W2A, DFF - W2A)], w2_v.at[pl.ds(W2A, DFF - W2A)])],
    ]

    def copies(g):
        return [pltpu.make_async_copy(src, dst, sems.at[g % NSEM])
                for src, dst in groups[g]]

    def start(g):
        if g < len(groups):
            for cp in copies(g):
                cp.start()

    def wait_and_refill(g):
        for cp in copies(g):
            cp.wait()
        start(g + NSEM)

    def to_smem(r):
        return pltpu.make_async_copy(
            wuv32.at[pl.ds(C_MAIN + r * SIDE_C, SIDE_C)], side_buf, side_sem)

    def to_vmem(r):
        return pltpu.make_async_copy(
            side_buf, slabs(wuv_v, C_MAIN + r * SIDE_C, SIDE_C), side_sem)

    for g in range(NSEM):
        start(g)
    to_smem(0).start()

    wait_and_refill(0)
    c = c_v[...].astype(F32)
    sc = (c * jax.nn.sigmoid(c)).astype(BF16)
    x0 = x_v[...].astype(F32)
    ln0 = _layernorm(x0)
    mod = _dot(sc, wmod_v[...])
    sa, ca, ga, sb, cb, gb = [mod[:, i * M:(i + 1) * M] for i in range(6)]
    h1 = (ln0 * (1.0 + ca) + sa).astype(BF16)
    to_smem(0).wait()
    to_vmem(0).start()

    wait_and_refill(1)
    to_vmem(0).wait()
    to_smem(1).start()

    def q_body(j, carry):
        lo, hi = _head_pair(wq_v, j)
        q_s[2 * j] = _dot(h1, lo).astype(BF16)
        q_s[2 * j + 1] = _dot(h1, hi).astype(BF16)
        return carry

    lax.fori_loop(0, NP, q_body, 0, unroll=UNROLL)

    wait_and_refill(2)
    to_smem(1).wait()
    to_vmem(1).start()

    def qa_body(j, carry):
        lo, hi = _head_pair(wuk_v, j)
        r0 = pl.multiple_of(2 * j * B, B)
        r1 = pl.multiple_of((2 * j + 1) * B, B)
        a0 = _dot_nt(q_s[2 * j], lo) * SCALE
        a1 = _dot_nt(q_s[2 * j + 1], hi) * SCALE
        for t in range(NCT):
            qa_s[t, pl.ds(r0, B), :] = a0[:, t * 128:(t + 1) * 128]
            qa_s[t, pl.ds(r1, B), :] = a1[:, t * 128:(t + 1) * 128]
        return carry

    lax.fori_loop(0, NP, qa_body, 0, unroll=UNROLL)

    def attn_body(b, carry):
        sem = sems.at[(KV0 + b) % NSEM]
        pltpu.make_async_copy(ckv_hbm.at[b], ckv_v.at[b], sem).wait()

        @pl.when(b + NSEM < B)
        def _():
            nb = b + NSEM
            pltpu.make_async_copy(ckv_hbm.at[nb], ckv_v.at[nb], sem).start()

        for i in range(NSEM):
            @pl.when(b == B - NSEM + i)
            def _():
                start(WUV + i)

        @pl.when(b % 2 == 0)
        def _():
            to_vmem(1 + b // 2).wait()
            to_smem(2 + b // 2).start()

        @pl.when(b % 2 == 1)
        def _():
            to_smem(2 + b // 2).wait()
            to_vmem(2 + b // 2).start()

        def attend(_, inner):
            qa = jnp.concatenate(
                [qa_s[t, pl.ds(b, H, stride=B), :] for t in range(NCT)],
                axis=-1).astype(BF16)
            kv = ckv_v[b]
            s = _dot_nt(qa, kv)
            m = jnp.max(s, axis=-1, keepdims=True)
            p = jnp.exp(s - m)
            l = jnp.sum(p, axis=-1, keepdims=True)
            cc = _dot(p.astype(BF16), kv) / l
            r0 = pl.multiple_of(b * H, H)
            for t in range(NCT):
                cc_s[t, pl.ds(r0, H), :] = cc[:, t * 128:(t + 1) * 128]
            return inner

        lax.fori_loop(0, jnp.minimum(b + 1, 1), attend, 0)
        return carry

    lax.fori_loop(0, B, attn_body, 0)

    wait_and_refill(WUV)
    to_vmem(SIDE - 1).wait()

    def ctx_body(j, carry):
        lo, hi = _head_pair(wuv_v, j)
        c0 = jnp.concatenate(
            [cc_s[t, pl.ds(2 * j, B, stride=H), :] for t in range(NCT)],
            axis=-1).astype(BF16)
        c1 = jnp.concatenate(
            [cc_s[t, pl.ds(2 * j + 1, B, stride=H), :] for t in range(NCT)],
            axis=-1).astype(BF16)
        ctx_s[2 * j] = _dot(c0, lo).astype(BF16)
        ctx_s[2 * j + 1] = _dot(c1, hi).astype(BF16)
        return carry

    lax.fori_loop(0, NP, ctx_body, 0, unroll=UNROLL)

    wait_and_refill(WUV + 1)
    ctx = jnp.concatenate([ctx_s[h] for h in range(H)], axis=-1)
    attn = _dot(ctx, wo_v[...])
    x1 = x0 + ga * attn

    h2 = (_layernorm(x1) * (1.0 + cb) + sb).astype(BF16)
    wait_and_refill(WUV + 2)
    f = jnp.maximum(_dot(h2, w1_v[...]), 0.0).astype(BF16)
    wait_and_refill(WUV + 3)
    acc_s[...] = x1 + gb * _dot(f[:, :W2A], w2_v[pl.ds(0, W2A), :])
    wait_and_refill(WUV + 4)
    x2 = acc_s[...] + gb * _dot(f[:, W2A:], w2_v[pl.ds(W2A, DFF - W2A), :])
    o_ref[...] = x2.astype(o_ref.dtype)


@jax.jit
def pallas_adaLN_cond__compressed_kv_cla__dense_activation_relu__decode_kernel(
    A_x: jax.Array,
    A_c_kv: jax.Array,
    A_w_q: jax.Array,
    A_w_uk: jax.Array,
    A_w_uv: jax.Array,
    A_w_o: jax.Array,
    B_x: jax.Array,
    B_w1: jax.Array,
    B_w2: jax.Array,
    c: jax.Array,
    w_mod: jax.Array,
):
    del B_x
    assert SIDE == (4 + B) // 2

    any_spec = pl.BlockSpec(memory_space=pl.ANY)
    scratch = [
        pltpu.VMEM((B, M), BF16),
        pltpu.VMEM((B, M), BF16),
        pltpu.VMEM((M, 6 * M), BF16),
        pltpu.VMEM((M, PITCH, D), U32),
        pltpu.VMEM((DC, PITCH, D), U32),
        pltpu.VMEM((B, SK, DC), BF16),
        pltpu.VMEM((DC, PITCH, D), U32),
        pltpu.VMEM((H * D, M), BF16),
        pltpu.VMEM((M, DFF), BF16),
        pltpu.VMEM((DFF, M), BF16),
        pltpu.VMEM((H, B, D), BF16),
        pltpu.VMEM((NCT, H * B, 128), F32),
        pltpu.VMEM((NCT, B * H, 128), F32),
        pltpu.VMEM((H, B, D), BF16),
        pltpu.VMEM((B, M), F32),
        pltpu.SemaphoreType.DMA((NSEM,)),
        pltpu.SMEM((SIDE_C, NP, D), U32),
        pltpu.SemaphoreType.DMA(()),
    ]
    out = pl.pallas_call(
        _kernel,
        out_shape=jax.ShapeDtypeStruct((B, M), BF16),
        in_specs=[any_spec] * 10,
        out_specs=pl.BlockSpec(memory_space=pltpu.VMEM),
        scratch_shapes=scratch,
        compiler_params=pltpu.CompilerParams(vmem_limit_bytes=100 * 1024 * 1024),
    )(A_x.reshape(B, M), A_c_kv, A_w_q, A_w_uk, A_w_uv,
      A_w_o.reshape(H * D, M), B_w1, B_w2, c, w_mod)
    return out.reshape(B, 1, M)
```

```python
import jax
import jax.numpy as jnp
from jax import lax
import jax.experimental.pallas as pl
import jax.experimental.pallas.tpu as pltpu

B = 8
SK = 4096
M = 512
DC = 512
H = 32
D = 128
DFF = 1792
NCT = DC // 128
NP = H // 2
EPS = 1e-05
SCALE = float(D) ** -0.5

W2A = 1536
PITCH = 24
UNROLL = 4
SIDE = 6
SIDE_C = 30
C_MAIN = DC - SIDE * SIDE_C
NGROUPS = 3 + B + 5

F32 = jnp.float32
BF16 = jnp.bfloat16
U32 = jnp.uint32


def _dot(a, b):
    return jnp.dot(a, b, preferred_element_type=F32)


def _dot_nt(a, b):
    return lax.dot_general(a, b, (((1,), (1,)), ((), ())),
                           preferred_element_type=F32)


def _layernorm(x):
    m = jnp.mean(x, axis=-1, keepdims=True)
    xc = x - m
    v = jnp.mean(xc * xc, axis=-1, keepdims=True)
    return xc / jnp.sqrt(v + EPS)


def _head_pair(w_ref, j):
    rows = w_ref.shape[0]
    flat = w_ref.reshape(rows * PITCH, D)
    words = flat[pl.ds(j, rows, stride=PITCH), :]
    lo = lax.bitcast_convert_type(words << 16, F32).astype(BF16)
    hi = lax.bitcast_convert_type(words & jnp.uint32(0xFFFF0000), F32).astype(BF16)
    return lo, hi


def _kernel(x_hbm, ckv_hbm, wq_hbm, wuk_hbm, wuv_hbm, wo_hbm, w1_hbm, w2_hbm,
            c_hbm, wmod_hbm,
            o_ref,
            x_v, c_v, wmod_v, wq_v, wuk_v, ckv_v, wuv_v, wo_v, w1_v, w2_v,
            q_s, qa_s, cc_s, ctx_s, acc_s, sems, side_buf, side_sem):
    wuv32 = wuv_hbm.bitcast(U32)

    def slabs(v, r0, n):
        return v.at[pl.ds(r0, n), pl.ds(0, NP), :]

    groups = [
        [(c_hbm, c_v), (x_hbm, x_v), (wmod_hbm, wmod_v)],
        [(wq_hbm.bitcast(U32), slabs(wq_v, 0, M))],
        [(wuk_hbm.bitcast(U32), slabs(wuk_v, 0, DC))],
    ]
    KV0 = len(groups)
    groups += [[(ckv_hbm.at[b], ckv_v.at[b])] for b in range(B)]
    WUV = len(groups)
    groups += [
        [(wuv32.at[pl.ds(0, C_MAIN)], slabs(wuv_v, 0, C_MAIN))],
        [(wo_hbm, wo_v)],
        [(w1_hbm, w1_v)],
        [(w2_hbm.at[pl.ds(0, W2A)], w2_v.at[pl.ds(0, W2A)])],
        [(w2_hbm.at[pl.ds(W2A, DFF - W2A)], w2_v.at[pl.ds(W2A, DFF - W2A)])],
    ]

    assert len(groups) == NGROUPS

    def copies(g):
        return [pltpu.make_async_copy(src, dst, sems.at[g])
                for src, dst in groups[g]]

    def wait(g):
        for cp in copies(g):
            cp.wait()

    def to_smem(r):
        return pltpu.make_async_copy(
            wuv32.at[pl.ds(C_MAIN + r * SIDE_C, SIDE_C)], side_buf, side_sem)

    def to_vmem(r):
        return pltpu.make_async_copy(
            side_buf, slabs(wuv_v, C_MAIN + r * SIDE_C, SIDE_C), side_sem)

    to_smem(0).start()
    for g in range(NGROUPS):
        for cp in copies(g):
            cp.start()

    wait(0)
    c = c_v[...].astype(F32)
    sc = (c * jax.nn.sigmoid(c)).astype(BF16)
    x0 = x_v[...].astype(F32)
    ln0 = _layernorm(x0)
    mod = _dot(sc, wmod_v[...])
    sa, ca, ga, sb, cb, gb = [mod[:, i * M:(i + 1) * M] for i in range(6)]
    h1 = (ln0 * (1.0 + ca) + sa).astype(BF16)
    to_smem(0).wait()
    to_vmem(0).start()

    wait(1)
    to_vmem(0).wait()
    to_smem(1).start()

    def q_body(j, carry):
        lo, hi = _head_pair(wq_v, j)
        q_s[2 * j] = _dot(h1, lo).astype(BF16)
        q_s[2 * j + 1] = _dot(h1, hi).astype(BF16)
        return carry

    lax.fori_loop(0, NP, q_body, 0, unroll=UNROLL)

    wait(2)
    to_smem(1).wait()
    to_vmem(1).start()

    def qa_body(j, carry):
        lo, hi = _head_pair(wuk_v, j)
        r0 = pl.multiple_of(2 * j * B, B)
        r1 = pl.multiple_of((2 * j + 1) * B, B)
        a0 = _dot_nt(q_s[2 * j], lo) * SCALE
        a1 = _dot_nt(q_s[2 * j + 1], hi) * SCALE
        for t in range(NCT):
            qa_s[t, pl.ds(r0, B), :] = a0[:, t * 128:(t + 1) * 128]
            qa_s[t, pl.ds(r1, B), :] = a1[:, t * 128:(t + 1) * 128]
        return carry

    lax.fori_loop(0, NP, qa_body, 0, unroll=UNROLL)

    def attn_body(b, carry):
        pltpu.make_async_copy(
            ckv_hbm.at[b], ckv_v.at[b], sems.at[KV0 + b]).wait()

        @pl.when(b % 2 == 0)
        def _():
            to_vmem(1 + b // 2).wait()
            to_smem(2 + b // 2).start()

        @pl.when(b % 2 == 1)
        def _():
            to_smem(2 + b // 2).wait()
            to_vmem(2 + b // 2).start()

        def attend(_, inner):
            qa = jnp.concatenate(
                [qa_s[t, pl.ds(b, H, stride=B), :] for t in range(NCT)],
                axis=-1).astype(BF16)
            kv = ckv_v[b]
            s = _dot_nt(qa, kv)
            m = jnp.max(s, axis=-1, keepdims=True)
            p = jnp.exp(s - m)
            l = jnp.sum(p, axis=-1, keepdims=True)
            cc = _dot(p.astype(BF16), kv) / l
            r0 = pl.multiple_of(b * H, H)
            for t in range(NCT):
                cc_s[t, pl.ds(r0, H), :] = cc[:, t * 128:(t + 1) * 128]
            return inner

        lax.fori_loop(0, jnp.minimum(b + 1, 1), attend, 0)
        return carry

    lax.fori_loop(0, B, attn_body, 0)

    wait(WUV)
    to_vmem(SIDE - 1).wait()

    def ctx_body(j, carry):
        lo, hi = _head_pair(wuv_v, j)
        c0 = jnp.concatenate(
            [cc_s[t, pl.ds(2 * j, B, stride=H), :] for t in range(NCT)],
            axis=-1).astype(BF16)
        c1 = jnp.concatenate(
            [cc_s[t, pl.ds(2 * j + 1, B, stride=H), :] for t in range(NCT)],
            axis=-1).astype(BF16)
        ctx_s[2 * j] = _dot(c0, lo).astype(BF16)
        ctx_s[2 * j + 1] = _dot(c1, hi).astype(BF16)
        return carry

    lax.fori_loop(0, NP, ctx_body, 0, unroll=UNROLL)

    wait(WUV + 1)
    ctx = jnp.concatenate([ctx_s[h] for h in range(H)], axis=-1)
    attn = _dot(ctx, wo_v[...])
    x1 = x0 + ga * attn

    h2 = (_layernorm(x1) * (1.0 + cb) + sb).astype(BF16)
    wait(WUV + 2)
    f = jnp.maximum(_dot(h2, w1_v[...]), 0.0).astype(BF16)
    wait(WUV + 3)
    acc_s[...] = x1 + gb * _dot(f[:, :W2A], w2_v[pl.ds(0, W2A), :])
    wait(WUV + 4)
    x2 = acc_s[...] + gb * _dot(f[:, W2A:], w2_v[pl.ds(W2A, DFF - W2A), :])
    o_ref[...] = x2.astype(o_ref.dtype)


@jax.jit
def pallas_adaLN_cond__compressed_kv_cla__dense_activation_relu__decode_kernel(
    A_x: jax.Array,
    A_c_kv: jax.Array,
    A_w_q: jax.Array,
    A_w_uk: jax.Array,
    A_w_uv: jax.Array,
    A_w_o: jax.Array,
    B_x: jax.Array,
    B_w1: jax.Array,
    B_w2: jax.Array,
    c: jax.Array,
    w_mod: jax.Array,
):
    del B_x
    assert SIDE == (4 + B) // 2

    any_spec = pl.BlockSpec(memory_space=pl.ANY)
    scratch = [
        pltpu.VMEM((B, M), BF16),
        pltpu.VMEM((B, M), BF16),
        pltpu.VMEM((M, 6 * M), BF16),
        pltpu.VMEM((M, PITCH, D), U32),
        pltpu.VMEM((DC, PITCH, D), U32),
        pltpu.VMEM((B, SK, DC), BF16),
        pltpu.VMEM((DC, PITCH, D), U32),
        pltpu.VMEM((H * D, M), BF16),
        pltpu.VMEM((M, DFF), BF16),
        pltpu.VMEM((DFF, M), BF16),
        pltpu.VMEM((H, B, D), BF16),
        pltpu.VMEM((NCT, H * B, 128), F32),
        pltpu.VMEM((NCT, B * H, 128), F32),
        pltpu.VMEM((H, B, D), BF16),
        pltpu.VMEM((B, M), F32),
        pltpu.SemaphoreType.DMA((NGROUPS,)),
        pltpu.SMEM((SIDE_C, NP, D), U32),
        pltpu.SemaphoreType.DMA(()),
    ]
    out = pl.pallas_call(
        _kernel,
        out_shape=jax.ShapeDtypeStruct((B, M), BF16),
        in_specs=[any_spec] * 10,
        out_specs=pl.BlockSpec(memory_space=pltpu.VMEM),
        scratch_shapes=scratch,
        compiler_params=pltpu.CompilerParams(
            vmem_limit_bytes=100 * 1024 * 1024,
            disable_semaphore_checks=True,
        ),
    )(A_x.reshape(B, M), A_c_kv, A_w_q, A_w_uk, A_w_uv,
      A_w_o.reshape(H * D, M), B_w1, B_w2, c, w_mod)
    return out.reshape(B, 1, M)
```

```python
import jax
import jax.numpy as jnp
from jax import lax
import jax.experimental.pallas as pl
import jax.experimental.pallas.tpu as pltpu

B = 8
SK = 4096
M = 512
DC = 512
H = 32
D = 128
DFF = 1792
NCT = DC // 128
NP = H // 2
EPS = 1e-05
SCALE = float(D) ** -0.5

W2_SPLIT = (0, 1280, 1664, DFF)
PITCH = 24
UNROLL = 4
SIDE = 6
SIDE_C = 30
C_MAIN = DC - SIDE * SIDE_C
NGROUPS = 3 + B + 3 + len(W2_SPLIT) - 1

F32 = jnp.float32
BF16 = jnp.bfloat16
U32 = jnp.uint32


def _dot(a, b):
    return jnp.dot(a, b, preferred_element_type=F32)


def _dot_nt(a, b):
    return lax.dot_general(a, b, (((1,), (1,)), ((), ())),
                           preferred_element_type=F32)


def _layernorm(x):
    m = jnp.mean(x, axis=-1, keepdims=True)
    xc = x - m
    v = jnp.mean(xc * xc, axis=-1, keepdims=True)
    return xc / jnp.sqrt(v + EPS)


def _head_pair(w_ref, j):
    rows = w_ref.shape[0]
    flat = w_ref.reshape(rows * PITCH, D)
    words = flat[pl.ds(j, rows, stride=PITCH), :]
    lo = lax.bitcast_convert_type(words << 16, F32).astype(BF16)
    hi = lax.bitcast_convert_type(words & jnp.uint32(0xFFFF0000), F32).astype(BF16)
    return lo, hi


def _kernel(x_hbm, ckv_hbm, wq_hbm, wuk_hbm, wuv_hbm, wo_hbm, w1_hbm, w2_hbm,
            c_hbm, wmod_hbm,
            o_ref,
            x_v, c_v, wmod_v, wq_v, wuk_v, ckv_v, wuv_v, wo_v, w1_v, w2_v,
            q_s, qa_s, cc_s, ctx_s, acc_s, sems, side_buf, side_sem):
    wuv32 = wuv_hbm.bitcast(U32)

    def slabs(v, r0, n):
        return v.at[pl.ds(r0, n), pl.ds(0, NP), :]

    groups = [
        [(c_hbm, c_v), (x_hbm, x_v), (wmod_hbm, wmod_v)],
        [(wq_hbm.bitcast(U32), slabs(wq_v, 0, M))],
        [(wuk_hbm.bitcast(U32), slabs(wuk_v, 0, DC))],
    ]
    KV0 = len(groups)
    groups += [[(ckv_hbm.at[b], ckv_v.at[b])] for b in range(B)]
    WUV = len(groups)
    groups += [
        [(wuv32.at[pl.ds(0, C_MAIN)], slabs(wuv_v, 0, C_MAIN))],
        [(wo_hbm, wo_v)],
        [(w1_hbm, w1_v)],
    ]
    W2G = len(groups)
    w2_rows = [pl.ds(lo, hi - lo) for lo, hi in zip(W2_SPLIT[:-1], W2_SPLIT[1:])]
    groups += [[(w2_hbm.at[rows], w2_v.at[rows])] for rows in w2_rows]

    assert len(groups) == NGROUPS

    def copies(g):
        return [pltpu.make_async_copy(src, dst, sems.at[g])
                for src, dst in groups[g]]

    def wait(g):
        for cp in copies(g):
            cp.wait()

    def to_smem(r):
        return pltpu.make_async_copy(
            wuv32.at[pl.ds(C_MAIN + r * SIDE_C, SIDE_C)], side_buf, side_sem)

    def to_vmem(r):
        return pltpu.make_async_copy(
            side_buf, slabs(wuv_v, C_MAIN + r * SIDE_C, SIDE_C), side_sem)

    to_smem(0).start()
    for g in range(NGROUPS):
        for cp in copies(g):
            cp.start()

    wait(0)
    c = c_v[...].astype(F32)
    sc = (c * jax.nn.sigmoid(c)).astype(BF16)
    x0 = x_v[...].astype(F32)
    ln0 = _layernorm(x0)
    mod = _dot(sc, wmod_v[...])
    sa, ca, ga, sb, cb, gb = [mod[:, i * M:(i + 1) * M] for i in range(6)]
    h1 = (ln0 * (1.0 + ca) + sa).astype(BF16)
    to_smem(0).wait()
    to_vmem(0).start()

    wait(1)
    to_vmem(0).wait()
    to_smem(1).start()

    def q_body(j, carry):
        lo, hi = _head_pair(wq_v, j)
        q_s[2 * j] = _dot(h1, lo).astype(BF16)
        q_s[2 * j + 1] = _dot(h1, hi).astype(BF16)
        return carry

    lax.fori_loop(0, NP, q_body, 0, unroll=UNROLL)

    wait(2)
    to_smem(1).wait()
    to_vmem(1).start()

    def qa_body(j, carry):
        lo, hi = _head_pair(wuk_v, j)
        r0 = pl.multiple_of(2 * j * B, B)
        r1 = pl.multiple_of((2 * j + 1) * B, B)
        a0 = _dot_nt(q_s[2 * j], lo) * SCALE
        a1 = _dot_nt(q_s[2 * j + 1], hi) * SCALE
        for t in range(NCT):
            qa_s[t, pl.ds(r0, B), :] = a0[:, t * 128:(t + 1) * 128]
            qa_s[t, pl.ds(r1, B), :] = a1[:, t * 128:(t + 1) * 128]
        return carry

    lax.fori_loop(0, NP, qa_body, 0, unroll=UNROLL)

    def attn_body(b, carry):
        pltpu.make_async_copy(
            ckv_hbm.at[b], ckv_v.at[b], sems.at[KV0 + b]).wait()

        @pl.when(b % 2 == 0)
        def _():
            to_vmem(1 + b // 2).wait()
            to_smem(2 + b // 2).start()

        @pl.when(b % 2 == 1)
        def _():
            to_smem(2 + b // 2).wait()
            to_vmem(2 + b // 2).start()

        def attend(_, inner):
            qa = jnp.concatenate(
                [qa_s[t, pl.ds(b, H, stride=B), :] for t in range(NCT)],
                axis=-1).astype(BF16)
            kv = ckv_v[b]
            s = _dot_nt(qa, kv)
            m = jnp.max(s, axis=-1, keepdims=True)
            p = jnp.exp(s - m)
            l = jnp.sum(p, axis=-1, keepdims=True)
            cc = _dot(p.astype(BF16), kv) / l
            r0 = pl.multiple_of(b * H, H)
            for t in range(NCT):
                cc_s[t, pl.ds(r0, H), :] = cc[:, t * 128:(t + 1) * 128]
            return inner

        lax.fori_loop(0, jnp.minimum(b + 1, 1), attend, 0)
        return carry

    lax.fori_loop(0, B, attn_body, 0)

    wait(WUV)
    to_vmem(SIDE - 1).wait()

    def ctx_body(j, carry):
        lo, hi = _head_pair(wuv_v, j)
        c0 = jnp.concatenate(
            [cc_s[t, pl.ds(2 * j, B, stride=H), :] for t in range(NCT)],
            axis=-1).astype(BF16)
        c1 = jnp.concatenate(
            [cc_s[t, pl.ds(2 * j + 1, B, stride=H), :] for t in range(NCT)],
            axis=-1).astype(BF16)
        ctx_s[2 * j] = _dot(c0, lo).astype(BF16)
        ctx_s[2 * j + 1] = _dot(c1, hi).astype(BF16)
        return carry

    lax.fori_loop(0, NP, ctx_body, 0, unroll=UNROLL)

    wait(WUV + 1)
    ctx = jnp.concatenate([ctx_s[h] for h in range(H)], axis=-1)
    attn = _dot(ctx, wo_v[...])
    x1 = x0 + ga * attn

    h2 = (_layernorm(x1) * (1.0 + cb) + sb).astype(BF16)
    wait(WUV + 2)
    f = jnp.maximum(_dot(h2, w1_v[...]), 0.0).astype(BF16)
    acc = x1
    for i, rows in enumerate(w2_rows):
        wait(W2G + i)
        lo, hi = W2_SPLIT[i], W2_SPLIT[i + 1]
        acc = acc + gb * _dot(f[:, lo:hi], w2_v[rows, :])
        if i + 1 < len(w2_rows):
            acc_s[...] = acc
            acc = acc_s[...]
    o_ref[...] = acc.astype(o_ref.dtype)


@jax.jit
def pallas_adaLN_cond__compressed_kv_cla__dense_activation_relu__decode_kernel(
    A_x: jax.Array,
    A_c_kv: jax.Array,
    A_w_q: jax.Array,
    A_w_uk: jax.Array,
    A_w_uv: jax.Array,
    A_w_o: jax.Array,
    B_x: jax.Array,
    B_w1: jax.Array,
    B_w2: jax.Array,
    c: jax.Array,
    w_mod: jax.Array,
):
    del B_x
    assert SIDE == (4 + B) // 2

    any_spec = pl.BlockSpec(memory_space=pl.ANY)
    scratch = [
        pltpu.VMEM((B, M), BF16),
        pltpu.VMEM((B, M), BF16),
        pltpu.VMEM((M, 6 * M), BF16),
        pltpu.VMEM((M, PITCH, D), U32),
        pltpu.VMEM((DC, PITCH, D), U32),
        pltpu.VMEM((B, SK, DC), BF16),
        pltpu.VMEM((DC, PITCH, D), U32),
        pltpu.VMEM((H * D, M), BF16),
        pltpu.VMEM((M, DFF), BF16),
        pltpu.VMEM((DFF, M), BF16),
        pltpu.VMEM((H, B, D), BF16),
        pltpu.VMEM((NCT, H * B, 128), F32),
        pltpu.VMEM((NCT, B * H, 128), F32),
        pltpu.VMEM((H, B, D), BF16),
        pltpu.VMEM((B, M), F32),
        pltpu.SemaphoreType.DMA((NGROUPS,)),
        pltpu.SMEM((SIDE_C, NP, D), U32),
        pltpu.SemaphoreType.DMA(()),
    ]
    out = pl.pallas_call(
        _kernel,
        out_shape=jax.ShapeDtypeStruct((B, M), BF16),
        in_specs=[any_spec] * 10,
        out_specs=pl.BlockSpec(memory_space=pltpu.VMEM),
        scratch_shapes=scratch,
        compiler_params=pltpu.CompilerParams(
            vmem_limit_bytes=100 * 1024 * 1024,
            disable_semaphore_checks=True,
        ),
    )(A_x.reshape(B, M), A_c_kv, A_w_q, A_w_uk, A_w_uv,
      A_w_o.reshape(H * D, M), B_w1, B_w2, c, w_mod)
    return out.reshape(B, 1, M)
```
